```python
import os as _os
_os.environ.setdefault("JAX_PLATFORMS", "cpu")
import jax
import jax.numpy as jnp

def _softmax(x, axis=-1):
    return jax.nn.softmax(x, axis=axis)
def _gelu(x):
    return jax.nn.gelu(x, approximate=True)
def _silu(x):
    return jax.nn.silu(x)
def _sigmoid(x):
    return jax.nn.sigmoid(x)
def _layernorm(x, axis=-1, eps=1e-5):
    m = jnp.mean(x, axis=axis, keepdims=True)
    v = jnp.var(x, axis=axis, keepdims=True)
    return (x - m) / jnp.sqrt(v + eps)
def _scatter_add(tgt, idx, src, axis=0):
    return tgt.at[idx].add(src)
def _segment_sum(src, seg, n):
    return jax.ops.segment_sum(src, seg, n)
class _Rng:
    def __init__(self, key):
        self._k = key
    def _next(self):
        self._k, sub = jax.random.split(self._k)
        return sub
    def normal(self, shape):
        return jax.random.normal(self._next(), shape, dtype=jnp.bfloat16)
    def randint(self, lo, hi, shape):
        return jax.random.randint(self._next(), shape, lo, hi, dtype=jnp.int32)
    def uniform(self, shape, lo=0.0, hi=1.0):
        return jax.random.uniform(self._next(), shape, jnp.bfloat16, lo, hi)
    def permutation(self, n):
        return jax.random.permutation(self._next(), n)


kernel_name = 'standalone__gqa_softmax__near_ridge'

def setup_inputs():
    _rng = _Rng(jax.random.key(int.from_bytes(__import__("os").urandom(4), "little")))
    _w = (lambda a: (lambda t: t.astype(jnp.bfloat16) if jnp.issubdtype(t.dtype, jnp.floating) else t)(jnp.asarray(a)))
    B, Hq, Hkv, Sq, Sk, D = 8, 16, 8, 512, 512, 256
    return {
        "q": _w((lambda *s: _rng.normal(s) * 0.4)(B, Hq, Sq, D)),
        "k": _w((lambda *s: _rng.normal(s) * 0.4)(B, Hkv, Sk, D)),
        "v": _w((lambda *s: _rng.normal(s) * 0.05)(B, Hkv, Sk, D)),
    }

def reference(q, k, v):
    B, Hq, Sq, D = q.shape
    Hkv = k.shape[1]
    rep = Hq // Hkv
    k = jnp.repeat(k, rep, axis=1)
    v = jnp.repeat(v, rep, axis=1)
    scale = D ** -0.5
    scores = jnp.einsum("bhqd,bhkd->bhqk", q, k) * scale
    p = _softmax(scores, axis=-1)
    return jnp.einsum("bhqk,bhkd->bhqd", p, v)
```

```python
import functools

import jax
import jax.numpy as jnp
import jax.experimental.pallas as pl
import jax.experimental.pallas.tpu as pltpu

_LOG2E = 1.4426950408889634
_HEADS_PER_STEP = 2


def _attn_kernel(q_ref, k_ref, v_ref, o_ref, *, c):
    for h in range(q_ref.shape[0]):
        s = jax.lax.dot_general(
            q_ref[h], k_ref[h], (((1,), (1,)), ((), ())),
            preferred_element_type=jnp.float32)
        m = jnp.max(s, axis=-1, keepdims=True)
        p = jnp.exp2((s - m) * c)
        l = jnp.sum(p, axis=-1, keepdims=True)
        r = pl.reciprocal(l, approx=True)
        r = r + r * (1.0 - l * r)
        o = jnp.dot(p.astype(jnp.bfloat16), v_ref[h],
                    preferred_element_type=jnp.float32)
        o_ref[h] = (o * r).astype(o_ref.dtype)


@jax.jit
def pallas_standalone__gqa_softmax__near_ridge_kernel(
    q: jax.Array,
    k: jax.Array,
    v: jax.Array,
):
    B, Hq, Sq, D = q.shape
    Hkv, Sk = k.shape[1], k.shape[2]
    rep = Hq // Hkv
    G = B * Hkv
    hpb = _HEADS_PER_STEP
    q2 = q.reshape(G, rep * Sq, D)
    k2 = k.reshape(G, Sk, D)
    v2 = v.reshape(G, Sk, D)
    c = (D ** -0.5) * _LOG2E
    out = pl.pallas_call(
        functools.partial(_attn_kernel, c=c),
        grid=(G // hpb,),
        in_specs=[
            pl.BlockSpec((hpb, rep * Sq, D), lambda g: (g, 0, 0)),
            pl.BlockSpec((hpb, Sk, D), lambda g: (g, 0, 0)),
            pl.BlockSpec((hpb, Sk, D), lambda g: (g, 0, 0)),
        ],
        out_specs=pl.BlockSpec((hpb, rep * Sq, D), lambda g: (g, 0, 0)),
        out_shape=jax.ShapeDtypeStruct((G, rep * Sq, D), q.dtype),
        compiler_params=pltpu.CompilerParams(
            dimension_semantics=("parallel",),
            disable_bounds_checks=True,
            vmem_limit_bytes=100 * 1024 * 1024),
    )(q2, k2, v2)
    return out.reshape(B, Hq, Sq, D)
```

```python
import functools
import jax, jax.numpy as jnp
import jax.experimental.pallas as pl
import jax.experimental.pallas.tpu as pltpu

LOG2E = 1.4426950408889634

def make(plan=((1, 2), (2, 1), (4, 1), (8, 7)), vmem_mb=120, nobc=True, dep='ko', split=(256,256,256,256), nosc=True,
         defer=8, chunk1=1024, chunkl=1024):
    NH = 64
    assert sum(n * r for n, r in plan) == NH
    NB = sum(r for n, r in plan)
    def kernel(q_hbm, k_hbm, v_hbm, o_hbm, qb, kb, vb, zs, sem_in, sem_o, *, c):
        zs[0] = 0
        zs[1] = 0
        def vview(sl): return vb.at[sl, pl.ds(0, 512)] if dep == 'vo' else vb.at[sl]
        def kview(sl): return kb.at[sl, pl.ds(0, 512)] if dep == 'ko' else kb.at[sl]
        def oview(sl, r0=0, n=1024):
            if dep == 'vo': return vb.at[sl, pl.ds(512 + r0, n)]
            if dep == 'ko': return kb.at[sl, pl.ds(512 + r0, n)]
            return qb.at[sl, pl.ds(r0, n)]
        def in_copies(b, h0, n):
            sl = pl.ds(h0, n)
            return (pltpu.make_async_copy(k_hbm.at[sl], kview(sl), sem_in.at[0, b]),
                    pltpu.make_async_copy(q_hbm.at[sl], qb.at[sl], sem_in.at[1, b]),
                    pltpu.make_async_copy(v_hbm.at[sl], vview(sl), sem_in.at[2, b]))

        h0 = 0; b = 0
        for n, rpt in plan:
            for _ in range(rpt):
                for cp in in_copies(b, h0, n):
                    cp.start()
                h0 += n; b += 1

        def qk(h, r0, n):
            return jax.lax.dot_general(qb[h, pl.ds(r0, n)], kview(h)[...], (((1,), (1,)), ((), ())), preferred_element_type=jnp.float32)
        def sm_pv(h, s):
            m = jnp.max(s, axis=-1, keepdims=True)
            p = jnp.exp2((s - m) * c)
            l = jnp.sum(p, axis=-1, keepdims=True)
            o = jnp.dot(p.astype(jnp.bfloat16), vview(h)[...], preferred_element_type=jnp.float32)
            return o, l
        def fin(h, r0, o, l, z, z2, sp, dma=True):
            r = pl.reciprocal(l, approx=True)
            r = r + r * (1.0 - l * r)
            res = (o * r).astype(jnp.bfloat16)
            off = 0
            for n in sp:
                oview(h + z, r0 + off, n)[...] = res[off:off + n]
                if dma:
                    pltpu.make_async_copy(oview(h + (z2 if len(sp) > 1 else z), r0 + off, n), o_hbm.at[h, pl.ds(r0 + off, n)], sem_o).start()
                off += n

        def block(b, h0, n, last_split, dma):
            for cp in in_copies(b, h0, n):
                cp.wait()
            z = zs[0]
            z2 = zs[1]
            units = []
            for j in range(n):
                ch = chunk1 if n == 1 else (chunkl if j == n - 1 else 1024)
                for r0 in range(0, 1024, ch):
                    units.append((h0 + j, r0, ch))
            prev = None
            for (h, r0, ch) in units:
                s = qk(h, r0, ch)
                if prev is not None:
                    fin(*prev, z, z2, (prev[2].shape[0],), dma)
                o, l = sm_pv(h, s)
                prev = (h, r0, o, l)
            ch = prev[2].shape[0]
            sp = last_split if (last_split and sum(last_split) == ch) else (ch,)
            fin(*prev, z, z2, sp, dma)

        h0 = 0; b = 0
        for n, rpt in plan:
            dma = h0 >= defer
            if h0 == defer and defer > 0:
                pltpu.make_async_copy(oview(pl.ds(0, defer)), o_hbm.at[pl.ds(0, defer)], sem_o).start()
            ls = split if h0 + n * rpt == NH else None
            if rpt == 1:
                block(b, h0, n, ls, dma)
            else:
                def body(g, carry, b=b, h0=h0, n=n, ls=ls, dma=dma):
                    block(b + g, h0 + g * n, n, ls, dma)
                    return carry
                jax.lax.fori_loop(0, rpt, body, 0)
            h0 += n * rpt; b += rpt
        pltpu.make_async_copy(o_hbm, o_hbm, sem_o).wait()

    @jax.jit
    def f(q, k, v):
        B, Hq, Sq, D = q.shape
        Hkv, Sk = k.shape[1], k.shape[2]
        rep = Hq // Hkv
        q2 = q.reshape(NH, rep * Sq, D)
        k2 = k.reshape(NH, Sk, D)
        v2 = v.reshape(NH, Sk, D)
        c = (D ** -0.5) * LOG2E
        out = pl.pallas_call(
            functools.partial(kernel, c=c),
            in_specs=[pl.BlockSpec(memory_space=pl.ANY)] * 3,
            out_specs=pl.BlockSpec(memory_space=pl.ANY),
            out_shape=jax.ShapeDtypeStruct((NH, rep * Sq, D), q.dtype),
            scratch_shapes=[
                pltpu.VMEM((NH, rep * Sq, D), q.dtype),
                pltpu.VMEM((NH, Sk + (rep * Sq if dep == 'ko' else 0), D), q.dtype),
                pltpu.VMEM((NH, Sk + (rep * Sq if dep == 'vo' else 0), D), q.dtype),
                pltpu.SMEM((2,), jnp.int32),
                pltpu.SemaphoreType.DMA((3, NB)),
                pltpu.SemaphoreType.DMA(()),
            ],
            compiler_params=pltpu.CompilerParams(
                disable_bounds_checks=nobc,
                disable_semaphore_checks=nosc,
                vmem_limit_bytes=vmem_mb * 1024 * 1024),
        )(q2, k2, v2)
        return out.reshape(B, Hq, Sq, D)
    return f


_f = make(chunk1=512,chunkl=512,split=(128,128,128,128))

@jax.jit
def pallas_standalone__gqa_softmax__near_ridge_kernel(q: jax.Array, k: jax.Array, v: jax.Array):
    return _f(q, k, v)
```

```python
import functools

import jax
import jax.numpy as jnp
import jax.experimental.pallas as pl
import jax.experimental.pallas.tpu as pltpu

_LOG2E = 1.4426950408889634
_RAMP_HEADS = 8
_GROUP = 8
_RAMP_OUT_ITER = 2
_TAIL_SPLIT = 4


def _attention_kernel(q_hbm, k_hbm, v_hbm, o_hbm, qb, kb, vob, zs, sem_in,
                      sem_out, *, c):
    nh, m_rows, _ = qb.shape
    sk = kb.shape[1]
    half = m_rows // 2
    n_groups = (nh - _RAMP_HEADS) // _GROUP

    zs[0] = 0
    zs[1] = 0

    def in_copy(desc, sem_idx):
        kind, h0, n_heads, r0, n_rows = desc
        src, dst = {"k": (k_hbm, kb), "q": (q_hbm, qb), "v": (v_hbm, vob)}[kind]
        return pltpu.make_async_copy(
            src.at[pl.ds(h0, n_heads), pl.ds(r0, n_rows)],
            dst.at[pl.ds(h0, n_heads), pl.ds(r0, n_rows)],
            sem_in.at[sem_idx])

    def group_descs(h0, n):
        return [("k", h0, n, 0, sk), ("q", h0, n, 0, m_rows), ("v", h0, n, 0, sk)]

    def o_stage(h, r0, n):
        return vob.at[h, pl.ds(sk + r0, n)]

    def run_ops(ops, env, h0, write_out):
        z, z2 = zs[0], zs[1]

        def get(kind, unit):
            j, r0, n = unit
            for k2, (j2, r2, n2), val in env:
                if k2 == kind and j2 == j and r2 <= r0 and r0 + n <= r2 + n2:
                    return val if n == n2 else val[r0 - r2:r0 - r2 + n]
            raise KeyError((kind, unit))

        for pos, (op, unit) in enumerate(ops):
            j, r0, n = unit
            h = h0 + j
            if op == "qk":
                s = jax.lax.dot_general(
                    qb[h, pl.ds(r0, n)], kb[h], (((1,), (1,)), ((), ())),
                    preferred_element_type=jnp.float32)
                env.append(("s", unit, s))
            elif op == "sm":
                s = get("s", unit)
                m = jnp.max(s, axis=-1, keepdims=True)
                p = jnp.exp2(s * c - m * c)
                env.append(("l", unit, jnp.sum(p, axis=-1, keepdims=True)))
                env.append(("p", unit, p.astype(jnp.bfloat16)))
            elif op == "pv":
                o = jnp.dot(get("p", unit), vob[h, pl.ds(0, sk)],
                            preferred_element_type=jnp.float32)
                env.append(("o", unit, o))
            else:
                l = get("l", unit)
                r = pl.reciprocal(l, approx=True)
                r = r + r * (1.0 - l * r)
                res = (get("o", unit) * r).astype(vob.dtype)
                parts = _TAIL_SPLIT if (write_out and pos == len(ops) - 1) else 1
                step = n // parts
                for i in range(parts):
                    rr = r0 + i * step
                    o_stage(h + z, rr, step)[...] = res[i * step:(i + 1) * step]
                    if write_out:
                        pltpu.make_async_copy(
                            o_stage(h + (z2 if parts > 1 else z), rr, step),
                            o_hbm.at[h, pl.ds(rr, step)], sem_out).start()

    def whole(units):
        return [(op, u) for u in units for op in ("qk", "sm", "pv", "fin")]

    def full(j):
        return (j, 0, m_rows)

    def lo(j):
        return (j, 0, half)

    def hi(j):
        return (j, half, half)

    def open_head(j):
        return [("qk", lo(j)), ("qk", hi(j)), ("sm", lo(j)), ("pv", lo(j)),
                ("sm", hi(j)), ("fin", lo(j))]

    def close_head(j):
        return [("pv", hi(j)), ("fin", hi(j))]

    ramp = [
        ([("k", 0, 1, 0, sk), ("q", 0, 1, 0, half)], open_head(0)[:1]),
        ([("q", 0, 1, half, half), ("v", 0, 1, 0, sk)], open_head(0)[1:]),
        (group_descs(1, 1), close_head(0) + open_head(1)),
        (group_descs(2, 2), close_head(1) + whole([full(2)]) + open_head(3)),
        (group_descs(4, 4), close_head(3) + whole([full(j) for j in range(4, 8)])),
    ]
    n_ramp_sems = sum(len(descs) for descs, _ in ramp)

    sem_idx = 0
    for descs, _ in ramp:
        for d in descs:
            in_copy(d, sem_idx).start()
            sem_idx += 1
    for g in range(n_groups):
        for d in group_descs(_RAMP_HEADS + g * _GROUP, _GROUP):
            in_copy(d, sem_idx).start()
            sem_idx += 1

    env = []
    sem_idx = 0
    for descs, ops in ramp:
        for d in descs:
            in_copy(d, sem_idx).wait()
            sem_idx += 1
        run_ops(ops, env, 0, write_out=False)

    def group_body(g, carry):
        h0 = _RAMP_HEADS + g * _GROUP
        for j, d in enumerate(group_descs(h0, _GROUP)):
            in_copy(d, n_ramp_sems + 3 * g + j).wait()

        @pl.when(g == _RAMP_OUT_ITER)
        def _():
            pltpu.make_async_copy(
                o_stage(pl.ds(0, _RAMP_HEADS), 0, m_rows),
                o_hbm.at[pl.ds(0, _RAMP_HEADS)], sem_out).start()

        last = _GROUP - 1
        units = [full(j) for j in range(last)] + [lo(last), hi(last)]
        run_ops(whole(units), [], h0, write_out=True)
        return carry

    jax.lax.fori_loop(0, n_groups, group_body, 0)

    pltpu.make_async_copy(o_hbm, o_hbm, sem_out).wait()


@jax.jit
def pallas_standalone__gqa_softmax__near_ridge_kernel(
    q: jax.Array,
    k: jax.Array,
    v: jax.Array,
):
    B, Hq, Sq, D = q.shape
    Hkv, Sk = k.shape[1], k.shape[2]
    rep = Hq // Hkv
    nh = B * Hkv
    m_rows = rep * Sq
    n_groups = (nh - _RAMP_HEADS) // _GROUP
    assert nh == _RAMP_HEADS + n_groups * _GROUP and n_groups > _RAMP_OUT_ITER
    assert m_rows % (32 * _TAIL_SPLIT) == 0 and Sk % 16 == 0

    out = pl.pallas_call(
        functools.partial(_attention_kernel, c=(D ** -0.5) * _LOG2E),
        in_specs=[pl.BlockSpec(memory_space=pl.ANY)] * 3,
        out_specs=pl.BlockSpec(memory_space=pl.ANY),
        out_shape=jax.ShapeDtypeStruct((nh, m_rows, D), q.dtype),
        scratch_shapes=[
            pltpu.VMEM((nh, m_rows, D), q.dtype),
            pltpu.VMEM((nh, Sk, D), k.dtype),
            pltpu.VMEM((nh, Sk + m_rows, D), v.dtype),
            pltpu.SMEM((2,), jnp.int32),
            pltpu.SemaphoreType.DMA((13 + 3 * n_groups,)),
            pltpu.SemaphoreType.DMA(()),
        ],
        compiler_params=pltpu.CompilerParams(
            disable_bounds_checks=True,
            disable_semaphore_checks=True,
            vmem_limit_bytes=110 * 1024 * 1024),
    )(q.reshape(nh, m_rows, D), k.reshape(nh, Sk, D), v.reshape(nh, Sk, D))
    return out.reshape(B, Hq, Sq, D)
```

```python
import functools

import jax
import jax.numpy as jnp
import jax.experimental.pallas as pl
import jax.experimental.pallas.tpu as pltpu

_LOG2E = 1.4426950408889634
_RAMP_HEADS = 8
_GROUP = 8
_RAMP_OUT_ITER = 2
_TAIL_SPLIT = 16
_N_RAMP_SEMS = 14
_NT_DIMS = (((1,), (1,)), ((), ()))


def _attention_kernel(q_hbm, k_hbm, v_hbm, o_hbm, qb, kb, vob, zs, sem_in,
                      sem_out, *, c):
    nh, m_rows, d = qb.shape
    sk = kb.shape[1]
    skt = sk // 2
    half, carry_rows = m_rows // 2, m_rows // 8
    n_groups = (nh - _RAMP_HEADS) // _GROUP

    zs[0] = 0
    zs[1] = 0

    def in_copy(desc, sem_idx):
        kind, h0, n_heads, r0, n_rows = desc
        src, dst = {"k": (k_hbm, kb), "q": (q_hbm, qb), "v": (v_hbm, vob)}[kind]
        return pltpu.make_async_copy(
            src.at[pl.ds(h0, n_heads), pl.ds(r0, n_rows)],
            dst.at[pl.ds(h0, n_heads), pl.ds(r0, n_rows)],
            sem_in.at[sem_idx])

    def k_desc(h0, n=1):
        return ("k", h0, n, 0, sk)

    def qv_descs(h0, n):
        return [("q", h0, n, 0, m_rows), ("v", h0, n, 0, sk)]

    def kqv_descs(h0, n):
        return [k_desc(h0, n)] + qv_descs(h0, n)

    def group_descs(h0):
        return [k_desc(h0 + 1, _GROUP - 1)] + qv_descs(h0, _GROUP)

    def o_stage(h, r0, n):
        return vob.at[h, pl.ds(sk + r0, n)]

    def kt_stage(slot):
        return vob.at[slot, pl.ds(0, d), pl.ds(0, skt)]

    def run_ops(ops, env, h0, write_out):
        z, z2 = zs[0], zs[1]

        def get(kind, unit):
            for k2, u2, val in env:
                if (k2, u2) == (kind, unit):
                    return val
            raise KeyError((kind, unit))

        for pos, (op, unit) in enumerate(ops):
            j, r0, n = unit
            h = h0 + j
            if op == "qk":
                s = jax.lax.dot_general(qb[h, pl.ds(r0, n)], kb[h], _NT_DIMS,
                                        preferred_element_type=jnp.float32)
                env.append(("s", unit, s))
            elif op == "qkt":
                q = qb[h, pl.ds(r0, n)]
                s0 = jnp.dot(q, kt_stage(nh)[...],
                             preferred_element_type=jnp.float32)
                s1 = jax.lax.dot_general(q, kb[h, pl.ds(skt, sk - skt)], _NT_DIMS,
                                         preferred_element_type=jnp.float32)
                env.append(("s", unit, jnp.concatenate([s0, s1], axis=1)))
            elif op == "kt":
                hn = h if isinstance(h, int) else jnp.minimum(h, nh - 1)
                kt_stage(nh + z)[...] = kb[hn, pl.ds(0, skt)].T
            elif op == "sm":
                s = get("s", unit)
                m = jnp.max(s, axis=-1, keepdims=True)
                p = jnp.exp2(s * c - m * c)
                env.append(("l", unit, jnp.sum(p, axis=-1, keepdims=True)))
                env.append(("p", unit, p.astype(jnp.bfloat16)))
            elif op == "pv":
                o = jnp.dot(get("p", unit), vob[h, pl.ds(0, sk)],
                            preferred_element_type=jnp.float32)
                env.append(("o", unit, o))
            else:
                l = get("l", unit)
                r = pl.reciprocal(l, approx=True)
                r = r + r * (1.0 - l * r)
                res = (get("o", unit) * r).astype(vob.dtype)
                parts = _TAIL_SPLIT if (write_out and pos == len(ops) - 1) else 1
                step = n // parts
                for i in range(parts):
                    rr = r0 + i * step
                    o_stage(h + z, rr, step)[...] = res[i * step:(i + 1) * step]
                    if write_out:
                        pltpu.make_async_copy(
                            o_stage(h + (z2 if parts > 1 else z), rr, step),
                            o_hbm.at[h, pl.ds(rr, step)], sem_out).start()

    def whole(units, use_kt=False, make_kt=None):
        ops = []
        for i, u in enumerate(units):
            ops += [("qkt" if use_kt and i == 0 else "qk", u), ("sm", u), ("pv", u)]
            if make_kt is not None and make_kt[0] == i:
                ops.append(("kt", (make_kt[1], 0, 0)))
            ops.append(("fin", u))
        return ops

    def full(j):
        return (j, 0, m_rows)

    def body_rows(j):
        return (j, 0, m_rows - carry_rows)

    def last_rows(j):
        return (j, m_rows - carry_rows, carry_rows)

    def open_head(j):
        a, b = body_rows(j), last_rows(j)
        return [("qk", a), ("qk", b), ("sm", a), ("pv", a), ("sm", b), ("fin", a)]

    def close_head(j):
        return [("pv", last_rows(j)), ("fin", last_rows(j))]

    a1, a2 = (0, 0, half - carry_rows), (0, half - carry_rows, carry_rows)
    b1, b2 = (0, half, half - carry_rows), last_rows(0)
    ramp = [
        ([k_desc(0), ("q", 0, 1, 0, half)],
         [("qk", a1), ("qk", a2), ("sm", a1)]),
        ([("q", 0, 1, half, half), ("v", 0, 1, 0, sk)],
         [("pv", a1), ("qk", b1), ("sm", a2), ("fin", a1), ("pv", a2), ("qk", b2),
          ("sm", b1), ("fin", a2), ("pv", b1), ("sm", b2), ("fin", b1)]),
        (kqv_descs(1, 1), close_head(0) + open_head(1)),
        (kqv_descs(2, 2), close_head(1) + whole([full(2)]) + open_head(3)),
        (kqv_descs(4, 4) + [k_desc(_RAMP_HEADS)],
         close_head(3) + whole([full(j) for j in range(4, _RAMP_HEADS)],
                               make_kt=(1, _RAMP_HEADS))),
    ]
    assert sum(len(descs) for descs, _ in ramp) == _N_RAMP_SEMS

    sem_idx = 0
    for descs, _ in ramp:
        for desc in descs:
            in_copy(desc, sem_idx).start()
            sem_idx += 1
    for g in range(n_groups):
        h0 = _RAMP_HEADS + g * _GROUP
        for j, desc in enumerate(group_descs(h0)):
            in_copy(desc, _N_RAMP_SEMS + 4 * g + j).start()
        if g + 1 < n_groups:
            in_copy(k_desc(h0 + _GROUP), _N_RAMP_SEMS + 4 * g + 3).start()

    env = []
    sem_idx = 0
    for descs, ops in ramp:
        for desc in descs:
            in_copy(desc, sem_idx).wait()
            sem_idx += 1
        run_ops(ops, env, 0, write_out=False)

    def group_body(g, carry):
        h0 = _RAMP_HEADS + g * _GROUP
        for j, desc in enumerate(group_descs(h0)):
            in_copy(desc, _N_RAMP_SEMS + 4 * g + j).wait()

        @pl.when(g + 1 < n_groups)
        def _():
            in_copy(k_desc(jnp.minimum(h0 + _GROUP, nh - 1)),
                    _N_RAMP_SEMS + 4 * g + 3).wait()

        @pl.when(g == _RAMP_OUT_ITER)
        def _():
            pltpu.make_async_copy(
                o_stage(pl.ds(0, _RAMP_HEADS), 0, m_rows),
                o_hbm.at[pl.ds(0, _RAMP_HEADS)], sem_out).start()

        last = _GROUP - 1
        units = [full(j) for j in range(last)] + [(last, 0, half), (last, half, half)]
        run_ops(whole(units, use_kt=True, make_kt=(3, _GROUP)), [], h0,
                write_out=True)
        return carry

    jax.lax.fori_loop(0, n_groups, group_body, 0)

    pltpu.make_async_copy(o_hbm, o_hbm, sem_out).wait()


@jax.jit
def pallas_standalone__gqa_softmax__near_ridge_kernel(
    q: jax.Array,
    k: jax.Array,
    v: jax.Array,
):
    B, Hq, Sq, D = q.shape
    Hkv, Sk = k.shape[1], k.shape[2]
    rep = Hq // Hkv
    nh = B * Hkv
    m_rows = rep * Sq
    n_groups = (nh - _RAMP_HEADS) // _GROUP
    assert nh == _RAMP_HEADS + n_groups * _GROUP and n_groups > _RAMP_OUT_ITER
    assert m_rows % (32 * _TAIL_SPLIT) == 0 and Sk % 32 == 0
    assert Sk // 2 <= D <= Sk + m_rows

    out = pl.pallas_call(
        functools.partial(_attention_kernel, c=(D ** -0.5) * _LOG2E),
        in_specs=[pl.BlockSpec(memory_space=pl.ANY)] * 3,
        out_specs=pl.BlockSpec(memory_space=pl.ANY),
        out_shape=jax.ShapeDtypeStruct((nh, m_rows, D), q.dtype),
        scratch_shapes=[
            pltpu.VMEM((nh, m_rows, D), q.dtype),
            pltpu.VMEM((nh, Sk, D), k.dtype),
            pltpu.VMEM((nh + 1, Sk + m_rows, D), v.dtype),
            pltpu.SMEM((2,), jnp.int32),
            pltpu.SemaphoreType.DMA((_N_RAMP_SEMS + 4 * n_groups,)),
            pltpu.SemaphoreType.DMA(()),
        ],
        compiler_params=pltpu.CompilerParams(
            disable_bounds_checks=True,
            disable_semaphore_checks=True,
            vmem_limit_bytes=110 * 1024 * 1024),
    )(q.reshape(nh, m_rows, D), k.reshape(nh, Sk, D), v.reshape(nh, Sk, D))
    return out.reshape(B, Hq, Sq, D)
```

```python
import functools

import jax
import jax.numpy as jnp
import jax.experimental.pallas as pl
import jax.experimental.pallas.tpu as pltpu

_LOG2E = 1.4426950408889634
_RAMP_HEADS = 8
_GROUP = 8
_RAMP_OUT_ITER = 2
_TAIL_SPLIT = 16
_N_RAMP_SEMS = 13
_NT_DIMS = (((1,), (1,)), ((), ()))


def _attention_kernel(q_hbm, k_hbm, v_hbm, o_hbm, qb, kb, vob, zs, sem_in,
                      sem_out, *, c):
    nh, m_rows, d = qb.shape
    sk = kb.shape[1]
    skt = sk // 2
    half, carry_rows = m_rows // 2, m_rows // 8
    n_groups = (nh - _RAMP_HEADS) // _GROUP

    zs[0] = 0
    zs[1] = 0

    def in_refs(desc):
        kind, h0, n_heads, r0, n_rows = desc
        src, dst = {"k": (k_hbm, kb), "q": (q_hbm, qb), "v": (v_hbm, vob)}[kind]
        idx = (pl.ds(h0, n_heads), pl.ds(r0, n_rows))
        return src, dst, idx

    def start_in(desc, sem_idx):
        src, dst, idx = in_refs(desc)
        pltpu.make_async_copy(src.at[idx], dst.at[idx], sem_in.at[sem_idx]).start()

    def wait_in(desc, sem_idx):
        _, dst, idx = in_refs(desc)
        pltpu.make_async_copy(dst.at[idx], dst.at[idx], sem_in.at[sem_idx]).wait()

    def k_desc(h0, n=1):
        return ("k", h0, n, 0, sk)

    def qv_descs(h0, n):
        return [("q", h0, n, 0, m_rows), ("v", h0, n, 0, sk)]

    def group_descs(h0):
        return [k_desc(h0 + 1, _GROUP)] + qv_descs(h0, _GROUP)

    def o_stage(h, r0, n):
        return vob.at[h, pl.ds(sk + r0, n)]

    def kt_stage(slot):
        return vob.at[slot, pl.ds(0, d), pl.ds(0, skt)]

    def run_ops(ops, env, h0, write_out):
        z, z2 = zs[0], zs[1]

        def get(kind, unit):
            for k2, u2, val in env:
                if (k2, u2) == (kind, unit):
                    return val
            raise KeyError((kind, unit))

        for pos, (op, unit) in enumerate(ops):
            j, r0, n = unit
            h = h0 + j
            if op == "qk":
                s = jax.lax.dot_general(qb[h, pl.ds(r0, n)], kb[h], _NT_DIMS,
                                        preferred_element_type=jnp.float32)
                env.append(("s", unit, s))
            elif op == "qkt":
                q = qb[h, pl.ds(r0, n)]
                s0 = jnp.dot(q, kt_stage(nh)[...],
                             preferred_element_type=jnp.float32)
                s1 = jax.lax.dot_general(q, kb[h, pl.ds(skt, sk - skt)], _NT_DIMS,
                                         preferred_element_type=jnp.float32)
                env.append(("s", unit, jnp.concatenate([s0, s1], axis=1)))
            elif op == "kt":
                kt_stage(nh + z)[...] = kb[h, pl.ds(0, skt)].T
            elif op == "sm":
                s = get("s", unit)
                m = jnp.max(s, axis=-1, keepdims=True)
                p = jnp.exp2(s * c - m * c)
                env.append(("l", unit, jnp.sum(p, axis=-1, keepdims=True)))
                env.append(("p", unit, p.astype(jnp.bfloat16)))
            elif op == "pv":
                o = jnp.dot(get("p", unit), vob[h, pl.ds(0, sk)],
                            preferred_element_type=jnp.float32)
                env.append(("o", unit, o))
            else:
                l = get("l", unit)
                r = pl.reciprocal(l, approx=True)
                r = r + r * (1.0 - l * r)
                res = (get("o", unit) * r).astype(vob.dtype)
                parts = _TAIL_SPLIT if (write_out and pos == len(ops) - 1) else 1
                step = n // parts
                for i in range(parts):
                    rr = r0 + i * step
                    o_stage(h + z, rr, step)[...] = res[i * step:(i + 1) * step]
                    if write_out:
                        pltpu.make_async_copy(
                            o_stage(h + (z2 if parts > 1 else z), rr, step),
                            o_hbm.at[h, pl.ds(rr, step)], sem_out).start()

    def whole(units, use_kt=False, make_kt=None):
        ops = []
        for i, u in enumerate(units):
            ops += [("qkt" if use_kt and i == 0 else "qk", u), ("sm", u), ("pv", u)]
            if make_kt is not None and make_kt[0] == i:
                ops.append(("kt", (make_kt[1], 0, 0)))
            ops.append(("fin", u))
        return ops

    def full(j):
        return (j, 0, m_rows)

    def body_rows(j):
        return (j, 0, m_rows - carry_rows)

    def last_rows(j):
        return (j, m_rows - carry_rows, carry_rows)

    def open_head(j):
        a, b = body_rows(j), last_rows(j)
        return [("qk", a), ("qk", b), ("sm", a), ("pv", a), ("sm", b), ("fin", a)]

    def close_head(j):
        return [("pv", last_rows(j)), ("fin", last_rows(j))]

    a1, a2 = (0, 0, half - carry_rows), (0, half - carry_rows, carry_rows)
    b1, b2 = (0, half, half - carry_rows), last_rows(0)
    ramp = [
        ([k_desc(0)], [("kt", (0, 0, 0))]),
        ([("q", 0, 1, 0, half)], [("qkt", a1), ("qk", a2), ("sm", a1)]),
        ([("q", 0, 1, half, half), ("v", 0, 1, 0, sk)],
         [("pv", a1), ("qk", b1), ("sm", a2), ("fin", a1), ("pv", a2), ("qk", b2),
          ("sm", b1), ("fin", a2), ("pv", b1), ("sm", b2), ("fin", b1)]),
        ([k_desc(1, 1)] + qv_descs(1, 1), close_head(0) + open_head(1)),
        ([k_desc(2, 2)] + qv_descs(2, 2),
         close_head(1) + whole([full(2)]) + open_head(3)),
        ([k_desc(4, 5)] + qv_descs(4, 4),
         close_head(3) + whole([full(j) for j in range(4, _RAMP_HEADS)],
                               make_kt=(1, _RAMP_HEADS))),
    ]
    assert sum(len(descs) for descs, _ in ramp) == _N_RAMP_SEMS

    sem_idx = 0
    for descs, _ in ramp:
        for desc in descs:
            start_in(desc, sem_idx)
            sem_idx += 1
    for g in range(n_groups):
        h0 = _RAMP_HEADS + g * _GROUP
        for j, desc in enumerate(group_descs(h0)):
            if j == 0 and g == n_groups - 1:
                start_in(k_desc(h0 + 1, _GROUP - 1), sem_idx)
                pltpu.make_async_copy(k_hbm.at[nh - 1], kb.at[nh],
                                      sem_in.at[sem_idx]).start()
            else:
                start_in(desc, sem_idx)
            sem_idx += 1

    env = []
    sem_idx = 0
    for descs, ops in ramp:
        for desc in descs:
            wait_in(desc, sem_idx)
            sem_idx += 1
        run_ops(ops, env, 0, write_out=False)

    def group_body(g, carry):
        h0 = _RAMP_HEADS + g * _GROUP
        for j, desc in enumerate(group_descs(h0)):
            wait_in(desc, _N_RAMP_SEMS + 3 * g + j)

        @pl.when(g == _RAMP_OUT_ITER)
        def _():
            pltpu.make_async_copy(
                o_stage(pl.ds(0, _RAMP_HEADS), 0, m_rows),
                o_hbm.at[pl.ds(0, _RAMP_HEADS)], sem_out).start()

        last = _GROUP - 1
        units = [full(j) for j in range(last)] + [(last, 0, half), (last, half, half)]
        run_ops(whole(units, use_kt=True, make_kt=(3, _GROUP)), [], h0,
                write_out=True)
        return carry

    jax.lax.fori_loop(0, n_groups, group_body, 0)

    pltpu.make_async_copy(o_hbm, o_hbm, sem_out).wait()


@jax.jit
def pallas_standalone__gqa_softmax__near_ridge_kernel(
    q: jax.Array,
    k: jax.Array,
    v: jax.Array,
):
    B, Hq, Sq, D = q.shape
    Hkv, Sk = k.shape[1], k.shape[2]
    rep = Hq // Hkv
    nh = B * Hkv
    m_rows = rep * Sq
    n_groups = (nh - _RAMP_HEADS) // _GROUP
    assert nh == _RAMP_HEADS + n_groups * _GROUP and n_groups > _RAMP_OUT_ITER
    assert m_rows % (32 * _TAIL_SPLIT) == 0 and Sk % 32 == 0
    assert Sk // 2 <= D <= Sk + m_rows

    out = pl.pallas_call(
        functools.partial(_attention_kernel, c=(D ** -0.5) * _LOG2E),
        in_specs=[pl.BlockSpec(memory_space=pl.ANY)] * 3,
        out_specs=pl.BlockSpec(memory_space=pl.ANY),
        out_shape=jax.ShapeDtypeStruct((nh, m_rows, D), q.dtype),
        scratch_shapes=[
            pltpu.VMEM((nh, m_rows, D), q.dtype),
            pltpu.VMEM((nh + 1, Sk, D), k.dtype),
            pltpu.VMEM((nh + 1, Sk + m_rows, D), v.dtype),
            pltpu.SMEM((2,), jnp.int32),
            pltpu.SemaphoreType.DMA((_N_RAMP_SEMS + 3 * n_groups,)),
            pltpu.SemaphoreType.DMA(()),
        ],
        compiler_params=pltpu.CompilerParams(
            disable_bounds_checks=True,
            disable_semaphore_checks=True,
            vmem_limit_bytes=110 * 1024 * 1024),
    )(q.reshape(nh, m_rows, D), k.reshape(nh, Sk, D), v.reshape(nh, Sk, D))
    return out.reshape(B, Hq, Sq, D)
```
